```python
import os as _os
_os.environ.setdefault("JAX_PLATFORMS", "cpu")
import jax
import jax.numpy as jnp

def _softmax(x, axis=-1):
    return jax.nn.softmax(x, axis=axis)
def _gelu(x):
    return jax.nn.gelu(x, approximate=True)
def _silu(x):
    return jax.nn.silu(x)
def _sigmoid(x):
    return jax.nn.sigmoid(x)
def _layernorm(x, axis=-1, eps=1e-5):
    m = jnp.mean(x, axis=axis, keepdims=True)
    v = jnp.var(x, axis=axis, keepdims=True)
    return (x - m) / jnp.sqrt(v + eps)
def _scatter_add(tgt, idx, src, axis=0):
    return tgt.at[idx].add(src)
def _segment_sum(src, seg, n):
    return jax.ops.segment_sum(src, seg, n)
class _Rng:
    def __init__(self, key):
        self._k = key
    def _next(self):
        self._k, sub = jax.random.split(self._k)
        return sub
    def normal(self, shape):
        return jax.random.normal(self._next(), shape, dtype=jnp.bfloat16)
    def randint(self, lo, hi, shape):
        return jax.random.randint(self._next(), shape, lo, hi, dtype=jnp.int32)
    def uniform(self, shape, lo=0.0, hi=1.0):
        return jax.random.uniform(self._next(), shape, jnp.bfloat16, lo, hi)
    def permutation(self, n):
        return jax.random.permutation(self._next(), n)


kernel_name = 'standalone__mha_softmax__near_ridge'

def setup_inputs():
    _rng = _Rng(jax.random.key(int.from_bytes(__import__("os").urandom(4), "little")))
    _w = (lambda a: (lambda t: t.astype(jnp.bfloat16) if jnp.issubdtype(t.dtype, jnp.floating) else t)(jnp.asarray(a)))
    B, H, Sq, Sk, D = 32, 32, 288, 512, 128
    return {
        "q": _w((lambda *s: _rng.normal(s) * 0.4)(B, H, Sq, D)),
        "k": _w((lambda *s: _rng.normal(s) * 0.4)(B, H, Sk, D)),
        "v": _w((lambda *s: _rng.normal(s) * 0.05)(B, H, Sk, D)),
    }

def reference(q, k, v):
    scale = q.shape[-1] ** -0.5
    scores = jnp.einsum("bhqd,bhkd->bhqk", q, k) * scale
    p = _softmax(scores, axis=-1)
    return jnp.einsum("bhqk,bhkd->bhqd", p, v)
```

```python
import math

import jax
import jax.numpy as jnp
from jax import lax
import jax.experimental.pallas as pl
import jax.experimental.pallas.tpu as pltpu


def _head(q, k, v, c):
    s = lax.dot_general(q, k, (((1,), (1,)), ((), ())), preferred_element_type=jnp.float32)
    m = jnp.max(s, axis=-1, keepdims=True)
    p = jnp.exp2((s - m) * c)
    l = jnp.sum(p, axis=-1, keepdims=True)
    o = jnp.dot(p.astype(jnp.bfloat16), v, preferred_element_type=jnp.float32)
    r = pl.reciprocal(l, approx=True)
    r = r * (2.0 - l * r)
    return o * r


@jax.jit
def pallas_standalone__mha_softmax__near_ridge_kernel(
    q: jax.Array,
    k: jax.Array,
    v: jax.Array,
):
    B, H, Sq, D = q.shape
    Sk = k.shape[2]
    N = B * H
    G, U = 16, 8
    c = (D ** -0.5) * math.log2(math.e)

    def kernel(q_ref, k_ref, v_ref, o_ref):
        def body(g, _):
            for u in range(U):
                h = g * U + u
                o_ref[h] = _head(q_ref[h], k_ref[h], v_ref[h], c).astype(o_ref.dtype)
            return 0

        lax.fori_loop(0, G // U, body, 0)

    out = pl.pallas_call(
        kernel,
        grid=(N // G,),
        in_specs=[
            pl.BlockSpec((G, Sq, D), lambda i: (i, 0, 0)),
            pl.BlockSpec((G, Sk, D), lambda i: (i, 0, 0)),
            pl.BlockSpec((G, Sk, D), lambda i: (i, 0, 0)),
        ],
        out_specs=pl.BlockSpec((G, Sq, D), lambda i: (i, 0, 0)),
        out_shape=jax.ShapeDtypeStruct((N, Sq, D), q.dtype),
        compiler_params=pltpu.CompilerParams(
            dimension_semantics=("parallel",),
            vmem_limit_bytes=100 * 1024 * 1024,
        ),
    )(q.reshape(N, Sq, D), k.reshape(N, Sk, D), v.reshape(N, Sk, D))
    return out.reshape(B, H, Sq, D)
```

```python
import math

import jax
import jax.numpy as jnp
from jax import lax
import jax.experimental.pallas as pl
import jax.experimental.pallas.tpu as pltpu

_G = 8
_NBUF = 8
_ROWS = 64
_S = 64
_NBLK = 4


def _attend(q, k, v, c):
    s = lax.dot_general(
        q, k, (((1,), (1,)), ((), ())), preferred_element_type=jnp.float32
    )
    m = jnp.max(s, axis=-1, keepdims=True)
    p = jnp.exp2((s - m) * c)
    l = jnp.sum(p, axis=-1, keepdims=True)
    o = jnp.dot(p.astype(v.dtype), v, preferred_element_type=jnp.float32)
    r = pl.reciprocal(l, approx=True)
    r = r * (2.0 - l * r)
    return o * r


@jax.jit
def pallas_standalone__mha_softmax__near_ridge_kernel(
    q: jax.Array,
    k: jax.Array,
    v: jax.Array,
):
    B, H, Sq, D = q.shape
    Sk = k.shape[2]
    N = B * H
    G, NBUF, ROWS, S, NBLK = _G, _NBUF, _ROWS, _S, _NBLK
    c = (D**-0.5) * math.log2(math.e)

    n = N // G
    slabs = (N * Sq) // (S * ROWS)
    n_win = slabs // NBLK
    blocks_per_step = (G * Sq) // ROWS
    j_last_read = n - NBUF
    assert n * G == N and slabs * S * ROWS == N * Sq and n_win * NBLK == slabs
    assert blocks_per_step * ROWS == G * Sq and j_last_read > 0
    assert NBUF <= n_win
    for t in range(NBUF):
        assert (t + 1) * NBLK * S * ROWS <= (j_last_read + t) * G * Sq

    def kernel(q_hbm, k_hbm, v_hbm, o_hbm, q_buf, k_buf, v_buf, o_buf, sem_in, sem_out):
        def reads(j, slot):
            heads = pl.ds(j * G, G)
            return [
                pltpu.make_async_copy(src.at[heads], dst.at[slot], sem_in.at[slot])
                for src, dst in ((q_hbm, q_buf), (k_hbm, k_buf), (v_hbm, v_buf))
            ]

        def start_window(w):
            def start_one(s, carry):
                win = pl.ds(w * NBLK, NBLK)
                pltpu.make_async_copy(
                    o_buf.at[win, s], o_hbm.at[win, s], sem_out
                ).start()
                return carry

            lax.fori_loop(0, S, start_one, 0)

        def store_head(j, u, o):
            pos = 0
            while pos < Sq:
                blk, off = divmod(u * Sq + pos, ROWS)
                cnt = min(ROWS - off, Sq - pos)
                b = j * blocks_per_step + blk
                o_buf[b // S, b % S, pl.ds(off, cnt), :] = o[pos : pos + cnt]
                pos += cnt

        for j in range(NBUF - 1):
            for cp in reads(j, j):
                cp.start()

        def step(j, carry):
            slot = j % NBUF

            @pl.when(j <= j_last_read)
            def _():
                for cp in reads(j + NBUF - 1, (j + NBUF - 1) % NBUF):
                    cp.start()

            @pl.when(j < j_last_read)
            def _():
                for cp in reads(j, slot):
                    cp.wait()

            @pl.when(j == j_last_read)
            def _():
                pending = [
                    cp for jj in range(j_last_read, n) for cp in reads(jj, jj % NBUF)
                ]
                for cp in pending[:-1]:
                    cp.wait()
                start_window(0)
                pending[-1].wait()

            @pl.when(j > j_last_read)
            def _():
                start_window(j - j_last_read)

            for u in range(G):
                o = _attend(q_buf[slot, u], k_buf[slot, u], v_buf[slot, u], c)
                store_head(j, u, o.astype(o_buf.dtype))
            return carry

        lax.fori_loop(0, n, step, 0)

        def start_rest(w, carry):
            start_window(w)
            return carry

        lax.fori_loop(NBUF, n_win, start_rest, 0)
        pltpu.make_async_copy(o_buf, o_hbm, sem_out).wait()

    out = pl.pallas_call(
        kernel,
        in_specs=[pl.BlockSpec(memory_space=pl.ANY)] * 3,
        out_specs=pl.BlockSpec(memory_space=pl.ANY),
        out_shape=jax.ShapeDtypeStruct((slabs, S, ROWS, D), q.dtype),
        scratch_shapes=[
            pltpu.VMEM((NBUF, G, Sq, D), q.dtype),
            pltpu.VMEM((NBUF, G, Sk, D), k.dtype),
            pltpu.VMEM((NBUF, G, Sk, D), v.dtype),
            pltpu.VMEM((slabs, S, ROWS, D), q.dtype),
            pltpu.SemaphoreType.DMA((NBUF,)),
            pltpu.SemaphoreType.DMA(()),
        ],
        compiler_params=pltpu.CompilerParams(
            vmem_limit_bytes=112 * 1024 * 1024,
        ),
    )(q.reshape(N, Sq, D), k.reshape(N, Sk, D), v.reshape(N, Sk, D))
    return out.reshape(B, H, Sq, D)
```

```python
import math

import jax
import jax.numpy as jnp
from jax import lax
import jax.experimental.pallas as pl
import jax.experimental.pallas.tpu as pltpu

_G = 8
_M = 8
_NBUF = 4
_RD_HEADS = 4
_RD_ROWS = 48
_OB = 32
_SB = 128
_WR_BLOCKS = 2
_WR_SLABS = 6


def _attend(q, k, v, c):
    s = lax.dot_general(
        q, k, (((1,), (1,)), ((), ())), preferred_element_type=jnp.float32
    )
    m = jnp.max(s, axis=-1, keepdims=True)
    p = jnp.exp2((s - m) * c)
    l = jnp.sum(p, axis=-1, keepdims=True)
    o = jnp.dot(p.astype(v.dtype), v, preferred_element_type=jnp.float32)
    r = pl.reciprocal(l, approx=True)
    r = r * (2.0 - l * r)
    return o * r


def _row_pieces(total, max_rows, unit=16):
    parts = -(-total // max_rows)
    base, rem = divmod(total // unit, parts)
    sizes = [(base + (i < rem)) * unit for i in range(parts)]
    starts = [sum(sizes[:i]) for i in range(parts)]
    assert sum(sizes) == total and max(sizes) <= max_rows
    return list(zip(starts, sizes))


def _read_plan(sq, sk):
    def pieces(arr, rows):
        return [
            (arr, g0, r0, nr)
            for r0, nr in _row_pieces(rows, _RD_ROWS)
            for g0 in range(0, _G, _RD_HEADS)
        ]

    qs, ks, vs = pieces(0, sq), pieces(1, sk), pieces(2, sk)
    half = len(qs) // 2
    prio0, prio1 = ks + qs[:half], qs[half:] + vs
    assert len(prio0) == len(prio1)
    return [x for a, b in zip(prio0, prio1) for x in (a + (0,), b + (1,))]


@jax.jit
def pallas_standalone__mha_softmax__near_ridge_kernel(
    q: jax.Array,
    k: jax.Array,
    v: jax.Array,
):
    B, H, Sq, D = q.shape
    Sk = k.shape[2]
    N = B * H
    G, M, NBUF, OB, SB = _G, _M, _NBUF, _OB, _SB
    c = (D**-0.5) * math.log2(math.e)

    n = N // G
    groups = N // (G * M)
    look = NBUF - 1
    j_drain = n - look
    slabs = (N * Sq) // (SB * OB)
    n_win = slabs // _WR_SLABS
    blocks_per_head = Sq // OB
    assert groups * G * M == N and blocks_per_head * OB == Sq
    assert slabs * SB * OB == N * Sq and n_win * _WR_SLABS == slabs
    assert SB & (SB - 1) == 0 and look < n_win
    for t in range(look):
        assert (t + 1) * _WR_SLABS * SB * OB <= ((j_drain + t) // M) * G * M * Sq

    plan = _read_plan(Sq, Sk)
    per_head = -(-len(plan) // G)

    def kernel(q_hbm, k_hbm, v_hbm, o_hbm, q_buf, k_buf, v_buf, o_buf, sem_in, sem_out):
        hbm = (q_hbm, k_hbm, v_hbm)
        buf = (q_buf, k_buf, v_buf)

        def start_reads(j, pieces):
            slot, grp, m = j % NBUF, j // M, j % M
            for arr, g0, r0, nr, prio in pieces:
                heads, rows = pl.ds(g0, _RD_HEADS), pl.ds(r0, nr)
                pltpu.make_async_copy(
                    hbm[arr].at[grp, heads, m, rows],
                    buf[arr].at[slot, heads, rows],
                    sem_in.at[slot, arr],
                ).start(priority=prio)

        def wait_reads(j, arrays=(0, 1, 2)):
            slot = j % NBUF
            for arr in arrays:
                dst = buf[arr].at[slot]
                pltpu.make_async_copy(dst, dst, sem_in.at[slot, arr]).wait()

        def start_window(w):
            def start_one(s, carry):
                idx = (pl.ds(w * _WR_SLABS, _WR_SLABS), pl.ds(s * _WR_BLOCKS, _WR_BLOCKS))
                pltpu.make_async_copy(o_buf.at[idx], o_hbm.at[idx], sem_out).start()
                return carry

            lax.fori_loop(0, SB // _WR_BLOCKS, start_one, 0)

        def prologue(j, carry):
            start_reads(j, plan)
            return carry

        lax.fori_loop(0, look, prologue, 0)

        def step(j, carry):
            @pl.when(j < j_drain)
            def _():
                wait_reads(j)

            @pl.when(j == j_drain)
            def _():
                for jj in range(j_drain, n - 1):
                    wait_reads(jj)
                wait_reads(n - 1, (0, 1))
                start_window(0)
                wait_reads(n - 1, (2,))

            @pl.when(j > j_drain)
            def _():
                start_window(j - j_drain)

            slot = j % NBUF
            head0 = (j // M) * (G * M) + j % M
            for g in range(G):
                o = _attend(q_buf[slot, g], k_buf[slot, g], v_buf[slot, g], c)
                o = o.astype(o_buf.dtype)
                for i in range(blocks_per_head):
                    b = (head0 + g * M) * blocks_per_head + i
                    slab = lax.shift_right_logical(b, SB.bit_length() - 1)
                    o_buf[slab, b & (SB - 1)] = o[i * OB : (i + 1) * OB]

                @pl.when(j < j_drain)
                def _():
                    start_reads(j + look, plan[g * per_head : (g + 1) * per_head])

            return carry

        lax.fori_loop(0, n, step, 0)

        def start_rest(w, carry):
            start_window(w)
            return carry

        lax.fori_loop(look, n_win, start_rest, 0)
        pltpu.make_async_copy(o_buf, o_hbm, sem_out).wait()

    out = pl.pallas_call(
        kernel,
        in_specs=[pl.BlockSpec(memory_space=pl.ANY)] * 3,
        out_specs=pl.BlockSpec(memory_space=pl.ANY),
        out_shape=jax.ShapeDtypeStruct((slabs, SB, OB, D), q.dtype),
        scratch_shapes=[
            pltpu.VMEM((NBUF, G, Sq, D), q.dtype),
            pltpu.VMEM((NBUF, G, Sk, D), k.dtype),
            pltpu.VMEM((NBUF, G, Sk, D), v.dtype),
            pltpu.VMEM((slabs, SB, OB, D), q.dtype),
            pltpu.SemaphoreType.DMA((NBUF, 3)),
            pltpu.SemaphoreType.DMA(()),
        ],
        compiler_params=pltpu.CompilerParams(
            vmem_limit_bytes=100 * 1024 * 1024,
            disable_bounds_checks=True,
            disable_semaphore_checks=True,
        ),
    )(
        q.reshape(groups, G, M, Sq, D),
        k.reshape(groups, G, M, Sk, D),
        v.reshape(groups, G, M, Sk, D),
    )
    return out.reshape(B, H, Sq, D)
```

```python
import math

import jax
import jax.numpy as jnp
from jax import lax
import jax.experimental.pallas as pl
import jax.experimental.pallas.tpu as pltpu

_G = 8
_M = 8
_CH = 2
_NBUF = 8
_LOOK = 4
_KV_SPLIT = ((0, 2, 96), (2, 4, 48), (6, 2, 96))
_Q_SPLIT = ((0, 4, 48), (4, 4, 48))
_SLAB = 4096
_WR_ROWS = 64
_WR_SLABS = 6


def _attend(q, k, v, c):
    s = lax.dot_general(
        q, k, (((1,), (1,)), ((), ())), preferred_element_type=jnp.float32
    )
    m = jnp.max(s, axis=-1, keepdims=True)
    p = jnp.exp2((s - m) * c)
    l = jnp.sum(p, axis=-1, keepdims=True)
    o = jnp.dot(p.astype(v.dtype), v, preferred_element_type=jnp.float32)
    r = pl.reciprocal(l, approx=True)
    r = r * (2.0 - l * r)
    return o * r


def _pieces(arr, rows, split, unit=16):
    out = []
    for g0, ng, max_rows in split:
        parts = -(-rows // max_rows)
        base, rem = divmod(rows // unit, parts)
        r0 = 0
        for i in range(parts):
            nr = (base + (i < rem)) * unit
            out.append((arr, g0, ng, r0, nr))
            r0 += nr
        assert r0 == rows
    assert sum(ng for _, ng, _ in split) == _G
    return sorted(out, key=lambda p: (p[3] + p[4] / 2, p[1]))


def _read_plan(sq, sk):
    qs, ks, vs = _pieces(0, sq, _Q_SPLIT), _pieces(1, sk, _KV_SPLIT), _pieces(2, sk, _KV_SPLIT)
    half = len(qs) // 2
    prio0, prio1 = ks + qs[:half], qs[half:] + vs
    assert len(prio0) == len(prio1)
    return [x for a, b in zip(prio0, prio1) for x in (a + (0,), b + (1,))]


@jax.jit
def pallas_standalone__mha_softmax__near_ridge_kernel(
    q: jax.Array,
    k: jax.Array,
    v: jax.Array,
):
    B, H, Sq, D = q.shape
    Sk = k.shape[2]
    N = B * H
    G, M, CH, NBUF, LOOK, SLAB = _G, _M, _CH, _NBUF, _LOOK, _SLAB
    scale_log2e = (D**-0.5) * math.log2(math.e)

    n_chunks = N // G
    groups = N // (G * M)
    n_steps = n_chunks // CH
    t_drain = (n_chunks - LOOK) // CH
    slabs = (N * Sq) // SLAB
    n_win = slabs // _WR_SLABS
    assert groups * G * M == N and n_steps * CH == n_chunks
    assert LOOK % CH == 0 and LOOK + CH <= NBUF and 0 < t_drain
    assert slabs * SLAB == N * Sq and n_win * _WR_SLABS == slabs
    assert SLAB & (SLAB - 1) == 0 and SLAB % _WR_ROWS == 0 and Sq % 32 == 0
    assert LOOK < n_win
    for w in range(LOOK):
        done_heads = (((t_drain + w // CH) * CH) // M) * G * M
        assert (w + 1) * _WR_SLABS * SLAB <= done_heads * Sq

    plan = _read_plan(Sq, Sk)
    per_head = -(-len(plan) // G)
    cuts = []
    for g in range(G):
        heads = [(a * G + g) * M + m for a in range(groups) for m in range(M)]
        inner = {-h * Sq % SLAB for h in heads}
        cuts.append([0] + sorted(x for x in inner if 0 < x < Sq) + [Sq])

    def kernel(q_hbm, k_hbm, v_hbm, o_hbm, q_buf, k_buf, v_buf, o_buf, sem_in, sem_out):
        hbm = (q_hbm, k_hbm, v_hbm)
        buf = (q_buf, k_buf, v_buf)

        def start_reads(c, pieces):
            slot, grp, m = c % NBUF, c // M, c % M
            for arr, g0, ng, r0, nr, prio in pieces:
                heads, rows = pl.ds(g0, ng), pl.ds(r0, nr)
                pltpu.make_async_copy(
                    hbm[arr].at[grp, heads, m, rows],
                    buf[arr].at[slot, heads, rows],
                    sem_in.at[slot, arr],
                ).start(priority=prio)

        def wait_reads(c, arrays=(0, 1, 2)):
            slot = c % NBUF
            for arr in arrays:
                dst = buf[arr].at[slot]
                pltpu.make_async_copy(dst, dst, sem_in.at[slot, arr]).wait()

        def start_window(w):
            def start_one(s, carry):
                rows = pl.ds(pl.multiple_of(s * _WR_ROWS, _WR_ROWS), _WR_ROWS)
                idx = (pl.ds(w * _WR_SLABS, _WR_SLABS), rows)
                pltpu.make_async_copy(o_buf.at[idx], o_hbm.at[idx], sem_out).start()
                return carry

            lax.fori_loop(0, SLAB // _WR_ROWS, start_one, 0)

        def prologue(c, carry):
            start_reads(c, plan)
            return carry

        lax.fori_loop(0, LOOK, prologue, 0)

        def step(t, carry):
            @pl.when(t < t_drain)
            def _():
                for i in range(CH):
                    wait_reads(t * CH + i)

            @pl.when(t == t_drain)
            def _():
                for c in range(t_drain * CH, n_chunks - 1):
                    wait_reads(c)
                wait_reads(n_chunks - 1, (0, 1))
                start_window(0)
                wait_reads(n_chunks - 1, (2,))
                for i in range(1, CH):
                    start_window(i)

            @pl.when(t > t_drain)
            def _():
                for i in range(CH):
                    start_window((t - t_drain) * CH + i)

            for i in range(CH):
                c = t * CH + i
                slot = c % NBUF
                head0 = (c // M) * (G * M) + c % M
                for g in range(G):
                    o = _attend(
                        q_buf[slot, g], k_buf[slot, g], v_buf[slot, g], scale_log2e
                    ).astype(o_buf.dtype)
                    row0 = (head0 + g * M) * Sq
                    for lo, hi in zip(cuts[g][:-1], cuts[g][1:]):
                        slab = lax.shift_right_logical(row0 + lo, SLAB.bit_length() - 1)
                        off = pl.multiple_of((row0 + lo) & (SLAB - 1), 32)
                        o_buf[slab, pl.ds(off, hi - lo), :] = o[lo:hi]

                    @pl.when(t < t_drain)
                    def _():
                        start_reads(c + LOOK, plan[g * per_head : (g + 1) * per_head])

            return carry

        lax.fori_loop(0, n_steps, step, 0)

        def start_rest(w, carry):
            start_window(w)
            return carry

        lax.fori_loop(LOOK, n_win, start_rest, 0)
        pltpu.make_async_copy(o_buf, o_hbm, sem_out).wait()

    out = pl.pallas_call(
        kernel,
        in_specs=[pl.BlockSpec(memory_space=pl.ANY)] * 3,
        out_specs=pl.BlockSpec(memory_space=pl.ANY),
        out_shape=jax.ShapeDtypeStruct((slabs, SLAB, D), q.dtype),
        scratch_shapes=[
            pltpu.VMEM((NBUF, G, Sq, D), q.dtype),
            pltpu.VMEM((NBUF, G, Sk, D), k.dtype),
            pltpu.VMEM((NBUF, G, Sk, D), v.dtype),
            pltpu.VMEM((slabs, SLAB, D), q.dtype),
            pltpu.SemaphoreType.DMA((NBUF, 3)),
            pltpu.SemaphoreType.DMA(()),
        ],
        compiler_params=pltpu.CompilerParams(
            vmem_limit_bytes=110 * 1024 * 1024,
            disable_bounds_checks=True,
            disable_semaphore_checks=True,
        ),
    )(
        q.reshape(groups, G, M, Sq, D),
        k.reshape(groups, G, M, Sk, D),
        v.reshape(groups, G, M, Sk, D),
    )
    return out.reshape(B, H, Sq, D)
```

```python
import math

import jax
import jax.numpy as jnp
from jax import lax
import jax.experimental.pallas as pl
import jax.experimental.pallas.tpu as pltpu

_G = 8
_M = 8
_ROT = 2
_CH = 2
_NBUF = 10
_LOOK = 8
_KV_SPLIT = ((0, 8, 16),)
_Q_SPLIT = ((0, 4, 48), (4, 4, 48))
_SLAB = 4096
_WR_ROWS = 64
_WR_SLABS = 6


def _attend(q, k, v, c):
    s = lax.dot_general(
        q, k, (((1,), (1,)), ((), ())), preferred_element_type=jnp.float32
    )
    m = jnp.max(s, axis=-1, keepdims=True)
    p = jnp.exp2((s - m) * c)
    l = jnp.sum(p, axis=-1, keepdims=True)
    o = jnp.dot(p.astype(v.dtype), v, preferred_element_type=jnp.float32)
    r = pl.reciprocal(l, approx=True)
    r = r * (2.0 - l * r)
    return o * r


def _read_plan(sq, sk):
    def pieces(arr, rows, split):
        assert sum(ng for _, ng, _ in split) == _G
        assert all(rows % nr == 0 for _, _, nr in split)
        out = [(arr, g0, ng, r0, nr) for g0, ng, nr in split for r0 in range(0, rows, nr)]
        return sorted(out, key=lambda p: (p[3], p[1]))

    qs, ks, vs = pieces(0, sq, _Q_SPLIT), pieces(1, sk, _KV_SPLIT), pieces(2, sk, _KV_SPLIT)
    half = len(qs) // 2
    prio0, prio1 = ks + qs[:half], qs[half:] + vs
    assert len(prio0) == len(prio1)
    return [x for a, b in zip(prio0, prio1) for x in (a + (0,), b + (1,))]


def _log2(x):
    assert x & (x - 1) == 0
    return x.bit_length() - 1


@jax.jit
def pallas_standalone__mha_softmax__near_ridge_kernel(
    q: jax.Array,
    k: jax.Array,
    v: jax.Array,
):
    B, H, Sq, D = q.shape
    Sk = k.shape[2]
    N = B * H
    G, M, CH, NBUF, LOOK, SLAB = _G, _M, _CH, _NBUF, _LOOK, _SLAB
    scale_log2e = (D**-0.5) * math.log2(math.e)

    n_rows = N // M
    wrap = G - _ROT
    n_chunks = N // G
    t_drain = (n_chunks - LOOK) // CH
    slabs = (N * Sq) // SLAB
    n_win = slabs // _WR_SLABS
    assert n_rows * M == N and n_rows % G == 0 and n_chunks % CH == 0
    assert LOOK == M and LOOK % CH == 0 and NBUF % CH == 0 and LOOK + CH <= NBUF
    assert slabs * SLAB == N * Sq and n_win * _WR_SLABS == slabs
    assert SLAB % _WR_ROWS == 0 and Sq % 32 == 0 and LOOK + 1 < n_win and t_drain > 0
    assert n_rows == 1 << _log2(n_rows)

    def head_of(c, g):
        return (((c // M) * G - wrap + g) % n_rows) * M + c % M

    for w in range(LOOK + 1):
        lo, hi = w * _WR_SLABS * SLAB, (w + 1) * _WR_SLABS * SLAB
        for c in range(t_drain * CH, n_chunks):
            for g in range(G):
                h = head_of(c, g)
                assert (h + 1) * Sq <= lo or h * Sq >= hi

    plan = _read_plan(Sq, Sk)
    per_head = -(-len(plan) // G)
    cuts = []
    for g in range(G):
        inner = {-head_of(c, g) * Sq % SLAB for c in range(n_chunks)}
        cuts.append([0] + sorted(x for x in inner if 0 < x < Sq) + [Sq])

    def kernel(q_hbm, k_hbm, v_hbm, o_hbm, q_buf, k_buf, v_buf, o_buf, sem_in, sem_out):
        hbm = (q_hbm, k_hbm, v_hbm)
        buf = (q_buf, k_buf, v_buf)

        def start_read(piece, row, col, slot, g0, ng):
            arr, _, _, r0, nr, prio = piece
            pltpu.make_async_copy(
                hbm[arr].at[pl.ds(row, ng), col, pl.ds(r0, nr)],
                buf[arr].at[slot, pl.ds(g0, ng), pl.ds(r0, nr)],
                sem_in.at[slot, arr],
            ).start(priority=prio)

        def wait_reads(slot, arrays=(0, 1, 2)):
            for arr in arrays:
                dst = buf[arr].at[slot]
                pltpu.make_async_copy(dst, dst, sem_in.at[slot, arr]).wait()

        def start_window(w):
            def start_one(s, carry):
                rows = pl.ds(pl.multiple_of(s * _WR_ROWS, _WR_ROWS), _WR_ROWS)
                idx = (pl.ds(w * _WR_SLABS, _WR_SLABS), rows)
                pltpu.make_async_copy(o_buf.at[idx], o_hbm.at[idx], sem_out).start()
                return carry

            lax.fori_loop(0, SLAB // _WR_ROWS, start_one, 0)

        def prologue(c, carry):
            for piece in plan:
                g0, g1 = piece[1], piece[1] + piece[2]
                if g0 < wrap:
                    start_read(piece, n_rows - wrap + g0, c, c, g0, min(g1, wrap) - g0)
                if g1 > wrap:
                    g0 = max(g0, wrap)
                    start_read(piece, g0 - wrap, c, c, g0, g1 - g0)
            return carry

        lax.fori_loop(0, LOOK, prologue, 0)

        def compute_chunk(c, slot, prefetch_slot=None):
            col = c & (M - 1)
            row = lax.shift_right_logical(c, _log2(M)) * G - wrap
            for g in range(G):
                o = _attend(
                    q_buf[slot, g], k_buf[slot, g], v_buf[slot, g], scale_log2e
                ).astype(o_buf.dtype)
                head = ((row + n_rows + g) & (n_rows - 1)) * M + col
                for lo, hi in zip(cuts[g][:-1], cuts[g][1:]):
                    r = head * Sq + lo
                    slab = lax.shift_right_logical(r, _log2(SLAB))
                    off = pl.multiple_of(r & (SLAB - 1), 32)
                    o_buf[slab, pl.ds(off, hi - lo), :] = o[lo:hi]
                if prefetch_slot is not None:
                    for piece in plan[g * per_head : (g + 1) * per_head]:
                        g0, ng = piece[1], piece[2]
                        start_read(piece, row + G + g0, col, prefetch_slot, g0, ng)

        def ring(slot):
            return jnp.where(slot >= NBUF, slot - NBUF, slot)

        def read_phase_step(t, slot0):
            for i in range(CH):
                wait_reads(slot0 + i)
            for i in range(CH):
                compute_chunk(t * CH + i, slot0 + i, ring(slot0 + i + LOOK))
            return ring(slot0 + CH)

        lax.fori_loop(0, t_drain, read_phase_step, 0)

        c_drain = t_drain * CH
        for c in range(c_drain, n_chunks - 1):
            wait_reads(c % NBUF)
        wait_reads((n_chunks - 1) % NBUF, (0, 1))
        start_window(0)
        wait_reads((n_chunks - 1) % NBUF, (2,))

        def write_phase_step(c, slot):
            start_window(c - c_drain + 1)
            compute_chunk(c, slot)
            return ring(slot + 1)

        lax.fori_loop(c_drain, n_chunks, write_phase_step, c_drain % NBUF)

        def start_rest(w, carry):
            start_window(w)
            return carry

        lax.fori_loop(LOOK + 1, n_win, start_rest, 0)
        pltpu.make_async_copy(o_buf, o_hbm, sem_out).wait()

    out = pl.pallas_call(
        kernel,
        in_specs=[pl.BlockSpec(memory_space=pl.ANY)] * 3,
        out_specs=pl.BlockSpec(memory_space=pl.ANY),
        out_shape=jax.ShapeDtypeStruct((slabs, SLAB, D), q.dtype),
        scratch_shapes=[
            pltpu.VMEM((NBUF, G, Sq, D), q.dtype),
            pltpu.VMEM((NBUF, G, Sk, D), k.dtype),
            pltpu.VMEM((NBUF, G, Sk, D), v.dtype),
            pltpu.VMEM((slabs, SLAB, D), q.dtype),
            pltpu.SemaphoreType.DMA((NBUF, 3)),
            pltpu.SemaphoreType.DMA(()),
        ],
        compiler_params=pltpu.CompilerParams(
            vmem_limit_bytes=120 * 1024 * 1024,
            disable_bounds_checks=True,
            disable_semaphore_checks=True,
        ),
    )(
        q.reshape(n_rows, M, Sq, D),
        k.reshape(n_rows, M, Sk, D),
        v.reshape(n_rows, M, Sk, D),
    )
    return out.reshape(B, H, Sq, D)
```

```python
import math

import jax
import jax.numpy as jnp
from jax import lax
import jax.experimental.pallas as pl
import jax.experimental.pallas.tpu as pltpu

_G = 8
_M = 8
_ROT = 2
_CH = 2
_NBUF = 10
_LOOK = 8
_KV_SPLIT = ((0, 8, 16),)
_Q_SPLIT = ((0, 4, 48), (4, 4, 48))
_SLAB = 4096
_WR_ROWS = 64
_WR_SLABS = 6


def _attend(q, k, v, c):
    s = lax.dot_general(
        q, k, (((1,), (1,)), ((), ())), preferred_element_type=jnp.float32
    )
    m = jnp.max(s, axis=-1, keepdims=True)
    p = jnp.exp2((s - m) * c)
    l = jnp.sum(p, axis=-1, keepdims=True)
    o = jnp.dot(p.astype(v.dtype), v, preferred_element_type=jnp.float32)
    r = pl.reciprocal(l, approx=True)
    r = r * (2.0 - l * r)
    return o * r


def _read_plan(sq, sk):
    def pieces(arr, rows, split):
        assert sum(ng for _, ng, _ in split) == _G
        assert all(rows % nr == 0 for _, _, nr in split)
        out = [(arr, g0, ng, r0, nr) for g0, ng, nr in split for r0 in range(0, rows, nr)]
        return sorted(out, key=lambda p: (p[3], p[1]))

    qs, ks, vs = pieces(0, sq, _Q_SPLIT), pieces(1, sk, _KV_SPLIT), pieces(2, sk, _KV_SPLIT)
    half = len(qs) // 2
    prio0, prio1 = ks + qs[:half], vs + qs[half:]
    assert len(prio0) == len(prio1)
    return [x for a, b in zip(prio0, prio1) for x in (a + (0,), b + (1,))]


def _log2(x):
    assert x & (x - 1) == 0
    return x.bit_length() - 1


@jax.jit
def pallas_standalone__mha_softmax__near_ridge_kernel(
    q: jax.Array,
    k: jax.Array,
    v: jax.Array,
):
    B, H, Sq, D = q.shape
    Sk = k.shape[2]
    N = B * H
    G, M, CH, NBUF, LOOK, SLAB = _G, _M, _CH, _NBUF, _LOOK, _SLAB
    scale_log2e = (D**-0.5) * math.log2(math.e)

    n_rows = N // M
    wrap = G - _ROT
    n_chunks = N // G
    t_drain = (n_chunks - LOOK) // CH
    slabs = (N * Sq) // SLAB
    n_win = slabs // _WR_SLABS
    assert n_rows * M == N and n_rows % G == 0 and n_chunks % CH == 0
    assert LOOK == M and LOOK % CH == 0 and NBUF % CH == 0 and LOOK + CH <= NBUF
    assert slabs * SLAB == N * Sq and n_win * _WR_SLABS == slabs
    assert SLAB % _WR_ROWS == 0 and Sq % 32 == 0 and LOOK + 1 < n_win and t_drain > 0
    assert n_rows == 1 << _log2(n_rows)

    def head_of(c, g):
        return (((c // M) * G - wrap + g) % n_rows) * M + c % M

    for w in range(LOOK + 1):
        lo, hi = w * _WR_SLABS * SLAB, (w + 1) * _WR_SLABS * SLAB
        for c in range(t_drain * CH, n_chunks):
            for g in range(G):
                h = head_of(c, g)
                assert (h + 1) * Sq <= lo or h * Sq >= hi

    plan = _read_plan(Sq, Sk)
    per_head = -(-len(plan) // G)
    cuts = []
    for g in range(G):
        inner = {-head_of(c, g) * Sq % SLAB for c in range(n_chunks)}
        cuts.append([0] + sorted(x for x in inner if 0 < x < Sq) + [Sq])

    def kernel(q_hbm, k_hbm, v_hbm, o_hbm, q_buf, k_buf, v_buf, o_buf, sem_in, sem_out):
        hbm = (q_hbm, k_hbm, v_hbm)
        buf = (q_buf, k_buf, v_buf)

        def start_read(piece, row, col, slot, g0, ng):
            arr, _, _, r0, nr, prio = piece
            pltpu.make_async_copy(
                hbm[arr].at[pl.ds(row, ng), col, pl.ds(r0, nr)],
                buf[arr].at[slot, pl.ds(g0, ng), pl.ds(r0, nr)],
                sem_in.at[slot, arr],
            ).start(priority=prio)

        def wait_reads(slot, arrays=(0, 1, 2)):
            for arr in arrays:
                dst = buf[arr].at[slot]
                pltpu.make_async_copy(dst, dst, sem_in.at[slot, arr]).wait()

        def start_window(w):
            def start_one(s, carry):
                rows = pl.ds(pl.multiple_of(s * _WR_ROWS, _WR_ROWS), _WR_ROWS)
                idx = (pl.ds(w * _WR_SLABS, _WR_SLABS), rows)
                pltpu.make_async_copy(o_buf.at[idx], o_hbm.at[idx], sem_out).start()
                return carry

            lax.fori_loop(0, SLAB // _WR_ROWS, start_one, 0)

        def prologue(c, carry):
            for piece in plan:
                g0, g1 = piece[1], piece[1] + piece[2]
                if g0 < wrap:
                    start_read(piece, n_rows - wrap + g0, c, c, g0, min(g1, wrap) - g0)
                if g1 > wrap:
                    g0 = max(g0, wrap)
                    start_read(piece, g0 - wrap, c, c, g0, g1 - g0)
            return carry

        lax.fori_loop(0, LOOK, prologue, 0)

        def compute_chunk(c, slot, prefetch_slot=None):
            col = c & (M - 1)
            row = lax.shift_right_logical(c, _log2(M)) * G - wrap
            for g in range(G):
                o = _attend(
                    q_buf[slot, g], k_buf[slot, g], v_buf[slot, g], scale_log2e
                ).astype(o_buf.dtype)
                head = ((row + n_rows + g) & (n_rows - 1)) * M + col
                for lo, hi in zip(cuts[g][:-1], cuts[g][1:]):
                    r = head * Sq + lo
                    slab = lax.shift_right_logical(r, _log2(SLAB))
                    off = pl.multiple_of(r & (SLAB - 1), 32)
                    o_buf[slab, pl.ds(off, hi - lo), :] = o[lo:hi]
                if prefetch_slot is not None:
                    for piece in plan[g * per_head : (g + 1) * per_head]:
                        g0, ng = piece[1], piece[2]
                        start_read(piece, row + G + g0, col, prefetch_slot, g0, ng)

        def ring(slot):
            return jnp.where(slot >= NBUF, slot - NBUF, slot)

        def read_phase_step(t, slot0):
            for i in range(CH):
                wait_reads(slot0 + i)
            for i in range(CH):
                compute_chunk(t * CH + i, slot0 + i, ring(slot0 + i + LOOK))
            return ring(slot0 + CH)

        lax.fori_loop(0, t_drain, read_phase_step, 0)

        c_drain = t_drain * CH
        for c in range(c_drain, n_chunks - 1):
            wait_reads(c % NBUF)
        wait_reads((n_chunks - 1) % NBUF, (1, 2))
        start_window(0)
        wait_reads((n_chunks - 1) % NBUF, (0,))

        def write_phase_step(c, slot):
            start_window(c - c_drain + 1)
            compute_chunk(c, slot)
            return ring(slot + 1)

        lax.fori_loop(c_drain, n_chunks, write_phase_step, c_drain % NBUF)

        def start_rest(w, carry):
            start_window(w)
            return carry

        lax.fori_loop(LOOK + 1, n_win, start_rest, 0)
        pltpu.make_async_copy(o_hbm, o_hbm, sem_out).wait()

    out = pl.pallas_call(
        kernel,
        in_specs=[pl.BlockSpec(memory_space=pl.ANY)] * 3,
        out_specs=pl.BlockSpec(memory_space=pl.ANY),
        out_shape=jax.ShapeDtypeStruct((slabs, SLAB, D), q.dtype),
        scratch_shapes=[
            pltpu.VMEM((NBUF, G, Sq, D), q.dtype),
            pltpu.VMEM((NBUF, G, Sk, D), k.dtype),
            pltpu.VMEM((NBUF, G, Sk, D), v.dtype),
            pltpu.VMEM((slabs, SLAB, D), q.dtype),
            pltpu.SemaphoreType.DMA((NBUF, 3)),
            pltpu.SemaphoreType.DMA(()),
        ],
        compiler_params=pltpu.CompilerParams(
            vmem_limit_bytes=112 * 1024 * 1024,
            disable_bounds_checks=True,
            disable_semaphore_checks=True,
        ),
    )(
        q.reshape(n_rows, M, Sq, D),
        k.reshape(n_rows, M, Sk, D),
        v.reshape(n_rows, M, Sk, D),
    )
    return out.reshape(B, H, Sq, D)
```
